```python
import os as _os
_os.environ.setdefault("JAX_PLATFORMS", "cpu")
import jax
import jax.numpy as jnp

def _softmax(x, axis=-1):
    return jax.nn.softmax(x, axis=axis)
def _gelu(x):
    return jax.nn.gelu(x, approximate=True)
def _silu(x):
    return jax.nn.silu(x)
def _sigmoid(x):
    return jax.nn.sigmoid(x)
def _layernorm(x, axis=-1, eps=1e-5):
    m = jnp.mean(x, axis=axis, keepdims=True)
    v = jnp.var(x, axis=axis, keepdims=True)
    return (x - m) / jnp.sqrt(v + eps)
def _scatter_add(tgt, idx, src, axis=0):
    return tgt.at[idx].add(src)
def _segment_sum(src, seg, n):
    return jax.ops.segment_sum(src, seg, n)
class _Rng:
    def __init__(self, key):
        self._k = key
    def _next(self):
        self._k, sub = jax.random.split(self._k)
        return sub
    def normal(self, shape):
        return jax.random.normal(self._next(), shape, dtype=jnp.bfloat16)
    def randint(self, lo, hi, shape):
        return jax.random.randint(self._next(), shape, lo, hi, dtype=jnp.int32)
    def uniform(self, shape, lo=0.0, hi=1.0):
        return jax.random.uniform(self._next(), shape, jnp.bfloat16, lo, hi)
    def permutation(self, n):
        return jax.random.permutation(self._next(), n)


kernel_name = 'parallel_sum__sliding_block_cached__dense_activation_mish__decode'

def setup_inputs():
    _rng = _Rng(jax.random.key(int.from_bytes(__import__("os").urandom(4), "little")))
    _w = (lambda a: (lambda t: t.astype(jnp.bfloat16) if jnp.issubdtype(t.dtype, jnp.floating) else t)(jnp.asarray(a)))
    def _A_setup():
        B, Sq, D = 2, 1, 512
        Hq, Hkv, Sk, Dh = 32, 8, 32768, 128
        assert Hq % Hkv == 0, (Hq, Hkv)
        return {
            "x": _w((lambda *s: _rng.normal(s) * 0.05)(B, Sq, D)),
            "k_cache": _w((lambda *s: _rng.normal(s) * 0.8)(B, Hkv, Sk, Dh)),
            "v_cache": _w((lambda *s: _rng.normal(s) * 0.8)(B, Hkv, Sk, Dh)),
            "wq": _w((lambda *s: _rng.normal(s) * 0.8)(D, Hq * Dh) * (D ** -0.5)),
            "wo": _w((lambda *s: _rng.normal(s) * 0.8)(Hq * Dh, D) * ((Hq * Dh) ** -0.5)),
        }
    _A_in = _A_setup()

    def _B_setup():
        B, S, D, F = 2, 1, 512, 1792
        return {
            "x": _w((lambda *s: _rng.normal(s) * 0.05)(B, S, D)),
            "w1": _w((lambda *s: _rng.normal(s) * 0.4)(D, F) * (D ** -0.5)),
            "b1": _w((lambda *s: _rng.normal(s) * 0.05)(F)),
            "w2": _w((lambda *s: _rng.normal(s) * 0.05)(F, D) * (F ** -0.5)),
        }
    _B_in = _B_setup()

    return {
        "A_x": _A_in["x"],
        "A_k_cache": _A_in["k_cache"],
        "A_v_cache": _A_in["v_cache"],
        "A_wq": _A_in["wq"],
        "A_wo": _A_in["wo"],
        "B_x": _B_in["x"],
        "B_w1": _B_in["w1"],
        "B_b1": _B_in["b1"],
        "B_w2": _B_in["w2"],
    }

def reference(A_x, A_k_cache, A_v_cache, A_wq, A_wo, B_x, B_w1, B_b1, B_w2):
    def _A_ref(x, k_cache, v_cache, wq, wo):
        B, Sq, D = x.shape
        Hq, Dh = 32, 128
        Hkv, Sk = k_cache.shape[1], k_cache.shape[2]
        W = min(4096, max(256, Sk // 4))
        rep = Hq // Hkv
        q = (lambda x, *d: x.transpose(*d))((x @ wq).reshape(B, Sq, Hq, Dh), 0, 2, 1, 3)
        k = jnp.repeat(k_cache[:, :, Sk - W:, :], rep, axis=1)
        v = jnp.repeat(v_cache[:, :, Sk - W:, :], rep, axis=1)
        scores = jnp.einsum("bhqd,bhkd->bhqk", q, k) * (Dh ** -0.5)
        p = _softmax(scores, axis=-1)
        o = jnp.einsum("bhqk,bhkd->bhqd", p, v)
        return (lambda x, *d: x.transpose(*d))(o, 0, 2, 1, 3).reshape(B, Sq, Hq * Dh) @ wo

    def _B_ref(x, w1, b1, w2):
        h = jnp.einsum("bsd,df->bsf", x, w1) + b1
        sp = jnp.log1p(jnp.exp(-jnp.abs(h))) + jnp.where(h > 0, h, jnp.zeros_like(h))
        act = h * jnp.tanh(sp)
        return jnp.einsum("bsf,fd->bsd", act, w2)

    x = A_x
    xn = _layernorm(x, axis=-1)
    return x + _A_ref(xn, A_k_cache, A_v_cache, A_wq, A_wo) + _B_ref(xn, B_w1, B_b1, B_w2)
```

```python
import jax
import jax.numpy as jnp
from jax import lax
import jax.experimental.pallas as pl
import jax.experimental.pallas.tpu as pltpu

HQ, DH = 32, 128
EPS = 1e-5
W2_CHUNKS = (8, 3, 2, 1)


def _kernel(x_hbm, k_hbm, v_hbm, wq_hbm, wo_hbm, w1_hbm, b1_hbm, w2_hbm, o_ref,
            xb, b1b, kbuf, vbuf, wqb, wob, w1b, w2b, qs, os_, sems):
    f32, bf16 = jnp.float32, jnp.bfloat16
    hkv, _, window, _ = kbuf.shape
    d, f = w1b.shape
    rep = HQ // hkv
    win = pl.ds(k_hbm.shape[2] - window, window)

    cp_x = pltpu.make_async_copy(x_hbm, xb, sems.at[0])
    cp_b1 = pltpu.make_async_copy(b1_hbm, b1b, sems.at[1])
    cp_w1 = pltpu.make_async_copy(w1_hbm, w1b, sems.at[2])
    cp_wq = pltpu.make_async_copy(wq_hbm, wqb, sems.at[3])
    cp_wo = pltpu.make_async_copy(wo_hbm, wob, sems.at[4])
    k0 = 5 + len(W2_CHUNKS)
    cp_k = lambda h: pltpu.make_async_copy(k_hbm.at[:, h, win, :], kbuf.at[h], sems.at[k0 + h])
    cp_v = lambda h: pltpu.make_async_copy(v_hbm.at[:, h, win, :], vbuf.at[h], sems.at[k0 + hkv + h])
    cp_w2, r0 = [], 0
    for i, n in enumerate(W2_CHUNKS):
        rows = pl.ds(r0 * 128, n * 128)
        cp_w2.append(pltpu.make_async_copy(w2_hbm.at[rows, :], w2b.at[rows, :], sems.at[5 + i]))
        r0 += n
    assert r0 * 128 == f

    cp_w1.start()
    cp_x.start()
    cp_b1.start()
    cp_wq.start()
    for h in range(hkv):
        cp_k(h).start()
        cp_v(h).start()
    cp_wo.start()
    for c in cp_w2:
        c.start()

    row = lax.broadcasted_iota(jnp.int32, (8, DH), 0)
    rowd = lax.broadcasted_iota(jnp.int32, (8, d), 0)

    cp_x.wait()
    x = xb[...].astype(f32)
    xc = x - jnp.mean(x, axis=-1, keepdims=True)
    var = jnp.mean(xc * xc, axis=-1, keepdims=True)
    xn = xc / jnp.sqrt(var + EPS)
    xr = jnp.where(rowd < rep, jnp.broadcast_to(xn[0:1], (8, d)), jnp.broadcast_to(xn[1:2], (8, d))).astype(bf16)

    cp_b1.wait()
    cp_w1.wait()
    hh = jnp.dot(xr, w1b[...], preferred_element_type=f32) + b1b[...].astype(f32).reshape(1, f)
    sp = jnp.log1p(jnp.exp(-jnp.abs(hh))) + jnp.maximum(hh, 0.0)
    act = hh * jnp.tanh(sp)
    rowf = lax.broadcasted_iota(jnp.int32, (8, f), 0)
    act = jnp.where(rowf % rep == 0, act, 0.0).astype(bf16)

    cp_wq.wait()

    def qproj(h, carry):
        cols = pl.ds(pl.multiple_of(h * (rep * DH), rep * DH), rep * DH)
        y = jnp.dot(xr, wqb[:, cols], preferred_element_type=f32)
        q = y[:, 0:DH]
        for r in range(1, rep):
            q = jnp.where(row % rep == r, y[:, r * DH:(r + 1) * DH], q)
        qs[h] = q
        return carry

    lax.fori_loop(0, hkv, qproj, 0)

    nt = (((1,), (1,)), ((), ()))

    def head(h, carry):
        q = qs[h].astype(bf16)
        cp_k(h).wait()
        s0 = lax.dot_general(q, kbuf[h, 0], nt, preferred_element_type=f32)
        s1 = lax.dot_general(q, kbuf[h, 1], nt, preferred_element_type=f32)
        roww = lax.broadcasted_iota(jnp.int32, (8, window), 0)
        s = jnp.where(roww < rep, s0, s1) * (DH ** -0.5)
        p = jnp.exp(s - jnp.max(s, axis=-1, keepdims=True))
        denom = jnp.sum(p, axis=-1, keepdims=True)
        pb = p.astype(bf16)
        cp_v(h).wait()
        o0 = jnp.dot(pb, vbuf[h, 0], preferred_element_type=f32)
        o1 = jnp.dot(pb, vbuf[h, 1], preferred_element_type=f32)
        os_[h] = jnp.where(row < rep, o0, o1) / denom
        return carry

    lax.fori_loop(0, hkv, head, 0)

    cp_wo.wait()

    def oproj(h, acc):
        o = os_[h]
        lhs = jnp.concatenate([jnp.where(row % rep == r, o, 0.0) for r in range(rep)], axis=1).astype(bf16)
        rows = pl.ds(pl.multiple_of(h * (rep * DH), rep * DH), rep * DH)
        return acc + jnp.dot(lhs, wob[rows, :], preferred_element_type=f32)

    acc = lax.fori_loop(0, hkv, oproj, jnp.zeros((8, d), f32))

    r0 = 0
    for i, n in enumerate(W2_CHUNKS):
        cp_w2[i].wait()
        acc = acc + jnp.dot(act[:, r0 * 128:(r0 + n) * 128], w2b[r0 * 128:(r0 + n) * 128, :],
                            preferred_element_type=f32)
        r0 += n
    res0 = jnp.sum(jnp.where(rowd < rep, acc, 0.0), axis=0, keepdims=True)
    res1 = jnp.sum(jnp.where(rowd >= rep, acc, 0.0), axis=0, keepdims=True)
    o_ref[...] = (x + jnp.concatenate([res0, res1], axis=0)).astype(o_ref.dtype)


@jax.jit
def pallas_parallel_sum__sliding_block_cached__dense_activation_mish__decode_kernel(
    A_x: jax.Array,
    A_k_cache: jax.Array,
    A_v_cache: jax.Array,
    A_wq: jax.Array,
    A_wo: jax.Array,
    B_x: jax.Array,
    B_w1: jax.Array,
    B_b1: jax.Array,
    B_w2: jax.Array,
):
    del B_x
    b, sq, d = A_x.shape
    _, hkv, sk, dh = A_k_cache.shape
    f = B_w1.shape[1]
    assert (b, sq, dh) == (2, 1, DH) and b * (HQ // hkv) == 8
    window = min(4096, max(256, sk // 4))
    hbm = pl.BlockSpec(memory_space=pl.ANY)
    out = pl.pallas_call(
        _kernel,
        in_specs=[hbm] * 8,
        out_specs=pl.BlockSpec(memory_space=pltpu.VMEM),
        out_shape=jax.ShapeDtypeStruct((b, d), A_x.dtype),
        scratch_shapes=[
            pltpu.VMEM((b, d), A_x.dtype),
            pltpu.VMEM((f,), B_b1.dtype),
            pltpu.VMEM((hkv, b, window, dh), A_k_cache.dtype),
            pltpu.VMEM((hkv, b, window, dh), A_v_cache.dtype),
            pltpu.VMEM(A_wq.shape, A_wq.dtype),
            pltpu.VMEM(A_wo.shape, A_wo.dtype),
            pltpu.VMEM(B_w1.shape, B_w1.dtype),
            pltpu.VMEM(B_w2.shape, B_w2.dtype),
            pltpu.VMEM((hkv, 8, dh), jnp.float32),
            pltpu.VMEM((hkv, 8, dh), jnp.float32),
            pltpu.SemaphoreType.DMA((5 + len(W2_CHUNKS) + 2 * hkv,)),
        ],
        compiler_params=pltpu.CompilerParams(vmem_limit_bytes=100 * 1024 * 1024),
    )(A_x.reshape(b, d), A_k_cache, A_v_cache, A_wq, A_wo, B_w1, B_b1, B_w2)
    return out.reshape(b, sq, d)
```

```python
import jax
import jax.numpy as jnp
from jax import lax
import jax.experimental.pallas as pl
import jax.experimental.pallas.tpu as pltpu

HQ, DH = 32, 128
EPS = 1e-5
KV_ROWS = (176, 176, 160)
W_ROWS = (48, 48, 32)
W1_ROWS, W2_ROWS = 16, 64
W2_BLOCKS = (8, 3, 2, 1)


def _kernel(x_hbm, k_hbm, v_hbm, wq_hbm, wo_hbm, w1_hbm, b1_hbm, w2_hbm, o_ref,
            xb, b1b, kb, vb, wqb, wob, w1b, w2b, sems):
    f32, bf16 = jnp.float32, jnp.bfloat16
    copy = pltpu.make_async_copy
    hkv, nb, window, _ = kb.shape
    d, f = w1b.shape
    rep = HQ // hkv
    g = rep * DH
    first = k_hbm.shape[2] - window
    sem_wq, sem_k, sem_v, sem_wo, sem_w2 = 0, 2, 4, 6, 8
    w2_start = [sum(W2_BLOCKS[:i]) * 128 for i in range(len(W2_BLOCKS) + 1)]
    assert w2_start[-1] == f

    def stream(n, pattern, pair):
        period = sum(pattern)
        assert n % period == 0

        def body(j, carry):
            off = 0
            for rows in pattern:
                lo, hi = pair(pl.multiple_of(j * period + off, 16), rows)
                lo.start(priority=1)
                hi.start(priority=0)
                off += rows
            return carry

        lax.fori_loop(0, n // period, body, 0)

    def fetch_head(h):
        cols = pl.ds(pl.multiple_of(h * g, g), g)
        stream(d // 2, W_ROWS, lambda r, n: [
            copy(wq_hbm.at[pl.ds(j * (d // 2) + r, n), cols], wqb.at[h, pl.ds(j * (d // 2) + r, n), :],
                 sems.at[sem_wq + h % 2]) for j in range(2)])
        for src, buf, sem in ((k_hbm, kb, sem_k), (v_hbm, vb, sem_v)):
            stream(window, KV_ROWS, lambda r, n, src=src, buf=buf, sem=sem: [
                copy(src.at[b, h, pl.ds(first + r, n), :], buf.at[h, b, pl.ds(r, n), :],
                     sems.at[sem + h % 2]) for b in range(nb)])
        stream(g // 2, W_ROWS, lambda r, n: [
            copy(wo_hbm.at[pl.ds(h * g + j * (g // 2) + r, n), :], wob.at[h, pl.ds(j * (g // 2) + r, n), :],
                 sems.at[sem_wo + h % 2]) for j in range(2)])

    def fetch_ffn():
        n1, n2 = d // W1_ROWS, f // W2_ROWS
        for _, is_w2, i in sorted([((i + 0.5) / n1, 0, i) for i in range(n1)]
                                  + [((i + 0.5) / n2, 1, i) for i in range(n2)]):
            if is_w2:
                rows = pl.ds(i * W2_ROWS, W2_ROWS)
                blk = max(j for j in range(len(W2_BLOCKS)) if w2_start[j] <= i * W2_ROWS)
                copy(w2_hbm.at[rows, :], w2b.at[rows, :], sems.at[sem_w2 + blk]).start(priority=1)
            else:
                rows = pl.ds(i * W1_ROWS, W1_ROWS)
                copy(w1_hbm.at[rows, :], w1b.at[rows, :], sems.at[sem_wq]).start(priority=0)

    def wait_filled(buf, sem):
        copy(buf, buf, sem).wait()

    cp_x = copy(x_hbm, xb, sems.at[sem_w2])
    cp_b1 = copy(b1_hbm, b1b, sems.at[sem_w2 + 1])
    cp_x.start()
    cp_b1.start()
    fetch_head(0)

    row = lax.broadcasted_iota(jnp.int32, (8, DH), 0)
    rowd = lax.broadcasted_iota(jnp.int32, (8, d), 0)
    cp_x.wait()
    cp_b1.wait()
    x = xb[...].astype(f32)
    xc = x - jnp.mean(x, axis=-1, keepdims=True)
    var = jnp.mean(xc * xc, axis=-1, keepdims=True)
    xn = xc / jnp.sqrt(var + EPS)
    xn0, xn1 = jnp.broadcast_to(xn[0:1], (8, d)), jnp.broadcast_to(xn[1:2], (8, d))
    xr = jnp.where(rowd < rep, xn0, xn1).astype(bf16)
    nt = (((1,), (1,)), ((), ()))

    def head(h, acc):
        par = h % 2
        pl.when(h + 1 < hkv)(lambda: fetch_head(h + 1))
        pl.when(h + 1 == hkv)(fetch_ffn)

        wait_filled(wqb.at[h], sems.at[sem_wq + par])
        y = jnp.dot(xr, wqb[h], preferred_element_type=f32)
        q = y[:, 0:DH]
        for r in range(1, rep):
            q = jnp.where(row % rep == r, y[:, r * DH:(r + 1) * DH], q)
        q = q.astype(bf16)

        wait_filled(kb.at[h], sems.at[sem_k + par])
        s0 = lax.dot_general(q, kb[h, 0], nt, preferred_element_type=f32)
        s1 = lax.dot_general(q, kb[h, 1], nt, preferred_element_type=f32)
        roww = lax.broadcasted_iota(jnp.int32, (8, window), 0)
        s = jnp.where(roww < rep, s0, s1) * (DH ** -0.5)
        p = jnp.exp(s - jnp.max(s, axis=-1, keepdims=True))
        denom = jnp.sum(p, axis=-1, keepdims=True)
        pb = p.astype(bf16)

        wait_filled(vb.at[h], sems.at[sem_v + par])
        o0 = jnp.dot(pb, vb[h, 0], preferred_element_type=f32)
        o1 = jnp.dot(pb, vb[h, 1], preferred_element_type=f32)
        o = jnp.where(row < rep, o0, o1) / denom
        lhs = jnp.concatenate([jnp.where(row % rep == r, o, 0.0) for r in range(rep)], axis=1).astype(bf16)

        wait_filled(wob.at[h], sems.at[sem_wo + par])
        return acc + jnp.dot(lhs, wob[h], preferred_element_type=f32)

    acc = lax.fori_loop(0, hkv, head, jnp.zeros((8, d), f32))
    res = x + jnp.concatenate([jnp.sum(jnp.where(rowd < rep, acc, 0.0), axis=0, keepdims=True),
                               jnp.sum(jnp.where(rowd >= rep, acc, 0.0), axis=0, keepdims=True)], axis=0)

    wait_filled(w1b, sems.at[sem_wq])
    hid = jnp.dot(jnp.where(rowd == 0, xn0, xn1).astype(bf16), w1b[...], preferred_element_type=f32)
    hid = hid + b1b[...].astype(f32).reshape(1, f)
    softplus = jnp.log1p(jnp.exp(-jnp.abs(hid))) + jnp.maximum(hid, 0.0)
    act = (hid * jnp.tanh(softplus)).astype(bf16)
    for i in range(len(W2_BLOCKS)):
        lo, hi = w2_start[i], w2_start[i + 1]
        wait_filled(w2b.at[pl.ds(lo, hi - lo), :], sems.at[sem_w2 + i])
        res = res + jnp.dot(act[:, lo:hi], w2b[lo:hi, :], preferred_element_type=f32)[0:nb]
    o_ref[...] = res.astype(o_ref.dtype)


@jax.jit
def pallas_parallel_sum__sliding_block_cached__dense_activation_mish__decode_kernel(
    A_x: jax.Array,
    A_k_cache: jax.Array,
    A_v_cache: jax.Array,
    A_wq: jax.Array,
    A_wo: jax.Array,
    B_x: jax.Array,
    B_w1: jax.Array,
    B_b1: jax.Array,
    B_w2: jax.Array,
):
    del B_x
    b, sq, d = A_x.shape
    _, hkv, sk, dh = A_k_cache.shape
    f = B_w1.shape[1]
    g = HQ // hkv * dh
    assert (b, sq, dh) == (2, 1, DH) and b * (HQ // hkv) == 8
    window = min(4096, max(256, sk // 4))
    hbm = pl.BlockSpec(memory_space=pl.ANY)
    out = pl.pallas_call(
        _kernel,
        in_specs=[hbm] * 8,
        out_specs=pl.BlockSpec(memory_space=pltpu.VMEM),
        out_shape=jax.ShapeDtypeStruct((b, d), A_x.dtype),
        scratch_shapes=[
            pltpu.VMEM((b, d), A_x.dtype),
            pltpu.VMEM((f,), B_b1.dtype),
            pltpu.VMEM((hkv, b, window, dh), A_k_cache.dtype),
            pltpu.VMEM((hkv, b, window, dh), A_v_cache.dtype),
            pltpu.VMEM((hkv, d, g), A_wq.dtype),
            pltpu.VMEM((hkv, g, d), A_wo.dtype),
            pltpu.VMEM(B_w1.shape, B_w1.dtype),
            pltpu.VMEM(B_w2.shape, B_w2.dtype),
            pltpu.SemaphoreType.DMA((8 + len(W2_BLOCKS),)),
        ],
        compiler_params=pltpu.CompilerParams(
            vmem_limit_bytes=100 * 1024 * 1024,
            disable_bounds_checks=True,
            disable_semaphore_checks=True,
        ),
    )(A_x.reshape(b, d), A_k_cache, A_v_cache, A_wq, A_wo, B_w1, B_b1, B_w2)
    return out.reshape(b, sq, d)
```

```python
import jax
import jax.numpy as jnp
from jax import lax
import jax.experimental.pallas as pl
import jax.experimental.pallas.tpu as pltpu

HQ, DH = 32, 128
EPS = 1e-5
KV_ROWS = (176, 176, 160)
W_ROWS = (48, 40, 40)
W1_ROWS, W2_ROWS = 16, 64
W2_BLOCKS = (8, 3, 2, 1)
PRIME = 4

SEM_WQ, SEM_K, SEM_V, SEM_WO, SEM_X, SEM_B1, SEM_W1, SEM_W2 = 0, 2, 4, 6, 8, 9, 10, 11


def _kernel(x_hbm, k_hbm, v_hbm, wq_hbm, wo_hbm, w1_hbm, b1_hbm, w2_hbm, o_ref,
            xb, b1b, kb, vb, wqb, wob, w1b, w2b):
    f32, bf16 = jnp.float32, jnp.bfloat16
    copy = pltpu.make_async_copy
    hkv, nb, window, _ = kb.shape
    d, f = w1b.shape
    rep = HQ // hkv
    g = rep * DH
    first = k_hbm.shape[2] - window
    kv_rows = KV_ROWS if window % sum(KV_ROWS) == 0 else (128,)
    w2_start = [sum(W2_BLOCKS[:i]) * 128 for i in range(len(W2_BLOCKS) + 1)]
    assert w2_start[-1] == f

    def stream(n, pattern, pair, periods=None, second_priority=0):
        period = sum(pattern)
        assert n % period == 0

        def body(j, carry):
            off = 0
            for rows in pattern:
                lo, hi = pair(pl.multiple_of(j * period + off, 8), rows)
                lo.start(priority=1)
                hi.start(priority=second_priority)
                off += rows
            return carry

        lax.fori_loop(*(periods or (0, n // period)), body, 0)

    def wait_filled(buf, sem):
        copy(buf, buf, sem).wait()

    def run(sems):
        def fetch_wq(h):
            cols = pl.ds(pl.multiple_of(h * g, g), g)
            stream(d // 2, W_ROWS, lambda r, n: [
                copy(wq_hbm.at[pl.ds(j * (d // 2) + r, n), cols],
                     wqb.at[h, pl.ds(j * (d // 2) + r, n), :],
                     sems.at[SEM_WQ + h % 2]) for j in range(2)])

        def fetch_kv(src, buf, sem, h, **kwargs):
            stream(window, kv_rows, lambda r, n: [
                copy(src.at[b, h, pl.ds(first + r, n), :],
                     buf.at[h, b, pl.ds(r, n), :],
                     sems.at[sem + h % 2]) for b in range(nb)], **kwargs)

        def fetch_wo(h):
            stream(g // 2, W_ROWS, lambda r, n: [
                copy(wo_hbm.at[pl.ds(h * g + j * (g // 2) + r, n), :],
                     wob.at[h, pl.ds(j * (g // 2) + r, n), :],
                     sems.at[SEM_WO + h % 2]) for j in range(2)])

        def fetch_head(h):
            fetch_wq(h)
            fetch_kv(k_hbm, kb, SEM_K, h)
            fetch_kv(v_hbm, vb, SEM_V, h)
            fetch_wo(h)

        def fetch_ffn():
            n1, n2 = d // W1_ROWS, f // W2_ROWS
            for _, is_w2, i in sorted([((i + 0.5) / n1, 0, i) for i in range(n1)]
                                      + [((i + 0.5) / n2, 1, i) for i in range(n2)]):
                if is_w2:
                    rows = pl.ds(i * W2_ROWS, W2_ROWS)
                    blk = max(j for j in range(len(W2_BLOCKS)) if w2_start[j] <= i * W2_ROWS)
                    copy(w2_hbm.at[rows, :], w2b.at[rows, :], sems.at[SEM_W2 + blk]).start(priority=1)
                else:
                    rows = pl.ds(i * W1_ROWS, W1_ROWS)
                    copy(w1_hbm.at[rows, :], w1b.at[rows, :], sems.at[SEM_W1]).start(priority=0)

        cp_x = copy(x_hbm, xb, sems.at[SEM_X])
        cp_b1 = copy(b1_hbm, b1b, sems.at[SEM_B1])
        periods = window // sum(kv_rows)
        prime = min(PRIME, periods)
        fetch_kv(k_hbm, kb, SEM_K, 0, periods=(0, prime), second_priority=1)
        fetch_wq(0)
        cp_x.start()
        cp_b1.start()
        fetch_kv(k_hbm, kb, SEM_K, 0, periods=(prime, periods))
        fetch_kv(v_hbm, vb, SEM_V, 0)
        fetch_wo(0)

        row = lax.broadcasted_iota(jnp.int32, (8, DH), 0)
        rowd = lax.broadcasted_iota(jnp.int32, (8, d), 0)
        cp_x.wait()
        cp_b1.wait()
        x = xb[...].astype(f32)
        xc = x - jnp.mean(x, axis=-1, keepdims=True)
        var = jnp.mean(xc * xc, axis=-1, keepdims=True)
        xn = xc / jnp.sqrt(var + EPS)
        xn0, xn1 = jnp.broadcast_to(xn[0:1], (8, d)), jnp.broadcast_to(xn[1:2], (8, d))

        xr = jnp.where(rowd < rep, xn0, xn1).astype(bf16)
        nt = (((1,), (1,)), ((), ()))

        def head(h, acc):
            par = h % 2
            pl.when(h + 1 < hkv)(lambda: fetch_head(h + 1))
            pl.when(h + 1 == hkv)(fetch_ffn)

            wait_filled(wqb.at[h], sems.at[SEM_WQ + par])
            wait_filled(kb.at[h], sems.at[SEM_K + par])
            y = jnp.dot(xr, wqb[h], preferred_element_type=f32)
            q = y[:, 0:DH]
            for r in range(1, rep):
                q = jnp.where(row % rep == r, y[:, r * DH:(r + 1) * DH], q)
            q = q.astype(bf16)
            s0 = lax.dot_general(q, kb[h, 0], nt, preferred_element_type=f32)
            s1 = lax.dot_general(q, kb[h, 1], nt, preferred_element_type=f32)
            roww = lax.broadcasted_iota(jnp.int32, (8, window), 0)
            s = jnp.where(roww < rep, s0, s1) * (DH ** -0.5)
            p = jnp.exp(s - jnp.max(s, axis=-1, keepdims=True))
            denom = jnp.sum(p, axis=-1, keepdims=True)
            pb = p.astype(bf16)

            wait_filled(vb.at[h], sems.at[SEM_V + par])
            o0 = jnp.dot(pb, vb[h, 0], preferred_element_type=f32)
            o1 = jnp.dot(pb, vb[h, 1], preferred_element_type=f32)
            o = jnp.where(row < rep, o0, o1) / denom
            lhs = jnp.concatenate([jnp.where(row % rep == r, o, 0.0) for r in range(rep)], axis=1)

            wait_filled(wob.at[h], sems.at[SEM_WO + par])
            return acc + jnp.dot(lhs.astype(bf16), wob[h], preferred_element_type=f32)

        acc = lax.fori_loop(0, hkv, head, jnp.zeros((8, d), f32))

        res0 = x[0:1] + jnp.sum(jnp.where(rowd < rep, acc, 0.0), axis=0, keepdims=True)
        res1 = x[1:2] + jnp.sum(jnp.where(rowd >= rep, acc, 0.0), axis=0, keepdims=True)
        res = jnp.where(rowd == 0, jnp.broadcast_to(res0, (8, d)), jnp.broadcast_to(res1, (8, d)))

        wait_filled(w1b, sems.at[SEM_W1])
        hid = jnp.dot(jnp.where(rowd == 0, xn0, xn1).astype(bf16), w1b[...], preferred_element_type=f32)
        hid = hid + b1b[...].astype(f32).reshape(1, f)
        softplus = jnp.log1p(jnp.exp(-jnp.abs(hid))) + jnp.maximum(hid, 0.0)
        act = (hid * jnp.tanh(softplus)).astype(bf16)
        for i in range(len(W2_BLOCKS)):
            lo, hi = w2_start[i], w2_start[i + 1]
            wait_filled(w2b.at[pl.ds(lo, hi - lo), :], sems.at[SEM_W2 + i])
            res = res + jnp.dot(act[:, lo:hi], w2b[lo:hi, :], preferred_element_type=f32)
        o_ref[...] = res.astype(o_ref.dtype)[0:nb]

    pl.run_scoped(run, pltpu.SemaphoreType.DMA((SEM_W2 + len(W2_BLOCKS),)))


@jax.jit
def pallas_parallel_sum__sliding_block_cached__dense_activation_mish__decode_kernel(
    A_x: jax.Array,
    A_k_cache: jax.Array,
    A_v_cache: jax.Array,
    A_wq: jax.Array,
    A_wo: jax.Array,
    B_x: jax.Array,
    B_w1: jax.Array,
    B_b1: jax.Array,
    B_w2: jax.Array,
):
    del B_x
    b, sq, d = A_x.shape
    _, hkv, sk, dh = A_k_cache.shape
    f = B_w1.shape[1]
    g = HQ // hkv * dh
    assert (b, sq, dh) == (2, 1, DH) and b * (HQ // hkv) == 8
    window = min(4096, max(256, sk // 4))
    hbm = pl.BlockSpec(memory_space=pl.ANY)
    out = pl.pallas_call(
        _kernel,
        in_specs=[hbm] * 8,
        out_specs=pl.BlockSpec(memory_space=pltpu.VMEM),
        out_shape=jax.ShapeDtypeStruct((b, d), A_x.dtype),
        scratch_shapes=[
            pltpu.VMEM((b, d), A_x.dtype),
            pltpu.VMEM((f,), B_b1.dtype),
            pltpu.VMEM((hkv, b, window, dh), A_k_cache.dtype),
            pltpu.VMEM((hkv, b, window, dh), A_v_cache.dtype),
            pltpu.VMEM((hkv, d, g), A_wq.dtype),
            pltpu.VMEM((hkv, g, d), A_wo.dtype),
            pltpu.VMEM(B_w1.shape, B_w1.dtype),
            pltpu.VMEM(B_w2.shape, B_w2.dtype),
        ],
        compiler_params=pltpu.CompilerParams(vmem_limit_bytes=100 * 1024 * 1024),
    )(A_x.reshape(b, d), A_k_cache, A_v_cache, A_wq, A_wo, B_w1, B_b1, B_w2)
    return out.reshape(b, sq, d)
```

```python
import functools

import jax
import jax.numpy as jnp
from jax import lax
import jax.experimental.pallas as pl
import jax.experimental.pallas.tpu as pltpu

HQ, DH = 32, 128
EPS = 1e-5
NR = 4
KV_ROWS = 32
W_ROWS = 8
W1_ROWS, W2_ROWS = 8, 32
W2_BLOCKS = (8, 3, 2, 1)
PRIME = 16

SEM_X, SEM_B1, SEM_WQ, SEM_K, SEM_V, SEM_WO, SEM_W1, SEM_W2 = 0, 1, 2, 3, 5, 7, 9, 10


def _kernel(x_hbm, k_hbm, v_hbm, wq_hbm, wo_hbm, w1_hbm, b1_hbm, w2_hbm, o_ref,
            xb, b1b, kb, vb, wqb, wob, w1b, w2b, q_scr, p_scr, l_scr, o_scr):
    f32, bf16 = jnp.float32, jnp.bfloat16
    copy = pltpu.make_async_copy
    groups, nb, _, window, _ = kb.shape
    hkv = groups * NR
    d, f = w1b.shape
    rep = HQ // hkv
    gw = rep * DH
    first = k_hbm.shape[2] - window
    kv_pairs = window // KV_ROWS // NR
    w2_start = [sum(W2_BLOCKS[:i]) * 128 for i in range(len(W2_BLOCKS) + 1)]
    assert w2_start[-1] == f and groups == 2 and kv_pairs * KV_ROWS * NR == window

    def start_pairs(lo, n, pair, second_priority=0):
        assert n % 2 == 0

        def body(j, carry):
            for u in range(2):
                a, b = pair(lo + 2 * j + u)
                a.start(priority=1)
                b.start(priority=second_priority)
            return carry

        lax.fori_loop(0, n // 2, body, 0)

    def wait_filled(buf, sem):
        copy(buf, buf, sem).wait()

    def run(sems):
        def wq_pair(i):
            rows = pl.ds(pl.multiple_of(i // (hkv // 2) * W_ROWS, W_ROWS), W_ROWS)
            heads = [i % (hkv // 2) + j * (hkv // 2) for j in range(2)]
            return [copy(wq_hbm.at[:, rows, pl.ds(pl.multiple_of(h * gw, gw), gw)],
                         wqb.at[h, :, rows, :], sems.at[SEM_WQ]) for h in heads]

        def kv_pair(src, buf, sem, g, i):
            off = pl.multiple_of(i * KV_ROWS, KV_ROWS)
            return [copy(src.at[b, pl.ds(g * NR, NR), pl.ds(first + off, KV_ROWS), :],
                         buf.at[g, b, :, pl.ds(off, KV_ROWS), :], sems.at[sem + g]) for b in range(nb)]

        def wo_pair(half, i):
            offs = [pl.multiple_of(j * (gw // 2) + i * W_ROWS, W_ROWS) for j in range(2)]
            return [copy(wo_hbm.at[:, pl.ds(half * gw + off, W_ROWS), :],
                         wob.at[half, :, pl.ds(off, W_ROWS), :], sems.at[SEM_WO + half]) for off in offs]

        def fetch_ffn(part):
            n1, n2 = d // W1_ROWS, f // W2_ROWS
            order = sorted([((i + 0.5) / n1, 0, i) for i in range(n1)]
                           + [((i + 0.5) / n2, 1, i) for i in range(n2)])
            for _, is_w2, i in order[part * (n1 + n2) // 2:(part + 1) * (n1 + n2) // 2]:
                if is_w2:
                    rows = pl.ds(i * W2_ROWS, W2_ROWS)
                    blk = max(j for j in range(len(W2_BLOCKS)) if w2_start[j] <= i * W2_ROWS)
                    copy(w2_hbm.at[rows, :], w2b.at[rows, :], sems.at[SEM_W2 + blk]).start(priority=1)
                else:
                    rows = pl.ds(i * W1_ROWS, W1_ROWS)
                    copy(w1_hbm.at[rows, :], w1b.at[rows, :], sems.at[SEM_W1]).start(priority=0)

        cp_x = copy(x_hbm, xb, sems.at[SEM_X])
        cp_b1 = copy(b1_hbm, b1b, sems.at[SEM_B1])
        start_pairs(0, PRIME, wq_pair, second_priority=1)
        cp_x.start()
        cp_b1.start()
        start_pairs(PRIME, d // NR // W_ROWS * hkv // 2 - PRIME, wq_pair)

        row = lax.broadcasted_iota(jnp.int32, (8, DH), 0)
        rowd = lax.broadcasted_iota(jnp.int32, (8, d), 0)
        cp_x.wait()
        cp_b1.wait()
        x = xb[...].astype(f32)
        xc = x - jnp.mean(x, axis=-1, keepdims=True)
        var = jnp.mean(xc * xc, axis=-1, keepdims=True)
        xn = xc / jnp.sqrt(var + EPS)
        xn0, xn1 = jnp.broadcast_to(xn[0:1], (8, d)), jnp.broadcast_to(xn[1:2], (8, d))

        xr = jnp.where(rowd < rep, xn0, xn1).astype(bf16)
        nt = (((1,), (1,)), ((), ()))

        def q_proj(h, carry):
            y = jnp.dot(xr, wqb[h].reshape(d, gw), preferred_element_type=f32)
            q = y[:, 0:DH]
            for r in range(1, rep):
                q = jnp.where(row % rep == r, y[:, r * DH:(r + 1) * DH], q)
            q_scr[h] = q
            return carry

        def scores(g, j):
            pl.when(j == 0)(lambda: wait_filled(kb.at[g], sems.at[SEM_K + g]))
            q = q_scr[g * NR + j].astype(bf16)
            s0 = lax.dot_general(q, kb[g, 0, j], nt, preferred_element_type=f32)
            s1 = lax.dot_general(q, kb[g, 1, j], nt, preferred_element_type=f32)
            roww = lax.broadcasted_iota(jnp.int32, (8, window), 0)
            s = jnp.where(roww < rep, s0, s1) * (DH ** -0.5)
            p = jnp.exp(s - jnp.max(s, axis=-1, keepdims=True))
            l_scr[j] = jnp.broadcast_to(jnp.sum(p, axis=-1, keepdims=True), (8, DH))
            p_scr[j] = p

        def values(g, j):
            pl.when(j == 0)(lambda: wait_filled(vb.at[g], sems.at[SEM_V + g]))
            p = p_scr[j].astype(bf16)
            o0 = jnp.dot(p, vb[g, 0, j], preferred_element_type=f32)
            o1 = jnp.dot(p, vb[g, 1, j], preferred_element_type=f32)
            o_scr[g * NR + j] = jnp.where(row < rep, o0, o1) / l_scr[j]

        kv_steps = 2 * hkv
        lag = NR + 1

        def step(i, carry):
            @pl.when(i < kv_steps)
            def _():
                g, lo = i // (2 * NR), i % NR * kv_pairs
                for which, (src, buf, sem) in enumerate(((k_hbm, kb, SEM_K), (v_hbm, vb, SEM_V))):
                    pl.when(i // NR % 2 == which)(functools.partial(
                        start_pairs, lo, kv_pairs, functools.partial(kv_pair, src, buf, sem, g)))

            pl.when((i >= kv_steps) & (i < kv_steps + 2))(lambda: start_pairs(
                0, gw // 2 // W_ROWS, functools.partial(wo_pair, i - kv_steps)))
            for part in range(2):
                pl.when(i == kv_steps + 2 + part)(functools.partial(fetch_ffn, part))

            @pl.when((i >= 1) & (i <= groups))
            def _():
                pl.when(i == 1)(lambda: wait_filled(wqb, sems.at[SEM_WQ]))
                lax.fori_loop((i - 1) * NR, i * NR, q_proj, 0)

            @pl.when(i >= lag)
            def _():
                u = i - lag
                for which, work in enumerate((scores, values)):
                    pl.when(u // NR % 2 == which)(functools.partial(work, u // (2 * NR), u % NR))

            return carry

        lax.fori_loop(0, kv_steps + lag, step, 0)

        def o_proj(t, acc):
            half, j = t // NR, t % NR
            pl.when(j == 0)(lambda: wait_filled(wob.at[half], sems.at[SEM_WO + half]))
            o = o_scr[2 * j + half]
            lhs = jnp.concatenate([jnp.where(row % rep == r, o, 0.0) for r in range(rep)], axis=1)
            return acc + jnp.dot(lhs.astype(bf16), wob[half, j], preferred_element_type=f32)

        acc = lax.fori_loop(0, hkv, o_proj, jnp.zeros((8, d), f32))

        res0 = x[0:1] + jnp.sum(jnp.where(rowd < rep, acc, 0.0), axis=0, keepdims=True)
        res1 = x[1:2] + jnp.sum(jnp.where(rowd >= rep, acc, 0.0), axis=0, keepdims=True)
        res = jnp.where(rowd == 0, jnp.broadcast_to(res0, (8, d)), jnp.broadcast_to(res1, (8, d)))

        wait_filled(w1b, sems.at[SEM_W1])
        hid = jnp.dot(jnp.where(rowd == 0, xn0, xn1).astype(bf16), w1b[...], preferred_element_type=f32)
        hid = hid + b1b[...].astype(f32).reshape(1, f)
        softplus = jnp.log1p(jnp.exp(-jnp.abs(hid))) + jnp.maximum(hid, 0.0)
        act = (hid * jnp.tanh(softplus)).astype(bf16)
        for i in range(len(W2_BLOCKS)):
            lo, hi = w2_start[i], w2_start[i + 1]
            wait_filled(w2b.at[pl.ds(lo, hi - lo), :], sems.at[SEM_W2 + i])
            res = res + jnp.dot(act[:, lo:hi], w2b[lo:hi, :], preferred_element_type=f32)
        o_ref[...] = res.astype(o_ref.dtype)[0:nb]

    pl.run_scoped(run, pltpu.SemaphoreType.DMA((SEM_W2 + len(W2_BLOCKS),)))


@jax.jit
def pallas_parallel_sum__sliding_block_cached__dense_activation_mish__decode_kernel(
    A_x: jax.Array,
    A_k_cache: jax.Array,
    A_v_cache: jax.Array,
    A_wq: jax.Array,
    A_wo: jax.Array,
    B_x: jax.Array,
    B_w1: jax.Array,
    B_b1: jax.Array,
    B_w2: jax.Array,
):
    del B_x
    b, sq, d = A_x.shape
    _, hkv, sk, dh = A_k_cache.shape
    f = B_w1.shape[1]
    gw = HQ // hkv * dh
    assert (b, sq, dh, hkv) == (2, 1, DH, 2 * NR)
    window = min(4096, max(256, sk // 4))
    hbm = pl.BlockSpec(memory_space=pl.ANY)
    out = pl.pallas_call(
        _kernel,
        in_specs=[hbm] * 8,
        out_specs=pl.BlockSpec(memory_space=pltpu.VMEM),
        out_shape=jax.ShapeDtypeStruct((b, d), A_x.dtype),
        scratch_shapes=[
            pltpu.VMEM((b, d), A_x.dtype),
            pltpu.VMEM((f,), B_b1.dtype),
            pltpu.VMEM((hkv // NR, b, NR, window, dh), A_k_cache.dtype),
            pltpu.VMEM((hkv // NR, b, NR, window, dh), A_v_cache.dtype),
            pltpu.VMEM((hkv, NR, d // NR, gw), A_wq.dtype),
            pltpu.VMEM((2, NR, gw, d), A_wo.dtype),
            pltpu.VMEM(B_w1.shape, B_w1.dtype),
            pltpu.VMEM(B_w2.shape, B_w2.dtype),
            pltpu.VMEM((hkv, 8, dh), jnp.float32),
            pltpu.VMEM((NR, 8, window), jnp.float32),
            pltpu.VMEM((NR, 8, dh), jnp.float32),
            pltpu.VMEM((hkv, 8, dh), jnp.float32),
        ],
        compiler_params=pltpu.CompilerParams(vmem_limit_bytes=100 * 1024 * 1024),
    )(A_x.reshape(b, d), A_k_cache, A_v_cache, A_wq.reshape(NR, d // NR, HQ * dh),
      A_wo.reshape(NR, HQ * dh // NR, d), B_w1, B_b1, B_w2)
    return out.reshape(b, sq, d)
```
